```python
import os as _os
_os.environ.setdefault("JAX_PLATFORMS", "cpu")
import jax
import jax.numpy as jnp

def _softmax(x, axis=-1):
    return jax.nn.softmax(x, axis=axis)
def _gelu(x):
    return jax.nn.gelu(x, approximate=True)
def _silu(x):
    return jax.nn.silu(x)
def _sigmoid(x):
    return jax.nn.sigmoid(x)
def _layernorm(x, axis=-1, eps=1e-5):
    m = jnp.mean(x, axis=axis, keepdims=True)
    v = jnp.var(x, axis=axis, keepdims=True)
    return (x - m) / jnp.sqrt(v + eps)
def _scatter_add(tgt, idx, src, axis=0):
    return tgt.at[idx].add(src)
def _segment_sum(src, seg, n):
    return jax.ops.segment_sum(src, seg, n)
class _Rng:
    def __init__(self, key):
        self._k = key
    def _next(self):
        self._k, sub = jax.random.split(self._k)
        return sub
    def normal(self, shape):
        return jax.random.normal(self._next(), shape, dtype=jnp.bfloat16)
    def randint(self, lo, hi, shape):
        return jax.random.randint(self._next(), shape, lo, hi, dtype=jnp.int32)
    def uniform(self, shape, lo=0.0, hi=1.0):
        return jax.random.uniform(self._next(), shape, jnp.bfloat16, lo, hi)
    def permutation(self, n):
        return jax.random.permutation(self._next(), n)


kernel_name = 'sequential_preLN__linear_attn_block__dense_activation_squared_relu__prompt'

def setup_inputs():
    _rng = _Rng(jax.random.key(int.from_bytes(__import__("os").urandom(4), "little")))
    _w = (lambda a: (lambda t: t.astype(jnp.bfloat16) if jnp.issubdtype(t.dtype, jnp.floating) else t)(jnp.asarray(a)))
    def _A_setup():
        B, S, D = 1, 2048, 576
        return {
            "x": _w((lambda *s: _rng.normal(s) * 0.05)(B, S, D)),
            "wqkv": _w((lambda *s: _rng.normal(s) * 0.1)(D, 3 * D)),
            "wo": _w((lambda *s: _rng.normal(s) * 0.05)(D, D)),
        }
    _A_in = _A_setup()

    def _B_setup():
        B, S, D, F = 1, 2048, 576, 4608
        return {
            "x": _w((lambda *s: _rng.normal(s) * 0.05)(B, S, D)),
            "w1": _w((lambda *s: _rng.normal(s) * 0.05)(D, F)),
            "b1": _w((lambda *s: _rng.normal(s) * 0.05)(F)),
            "w2": _w((lambda *s: _rng.normal(s) * 0.05)(F, D)),
            "b2": _w((lambda *s: _rng.normal(s) * 0.05)(D)),
        }
    _B_in = _B_setup()

    return {
        "A_x": _A_in["x"],
        "A_wqkv": _A_in["wqkv"],
        "A_wo": _A_in["wo"],
        "B_x": _B_in["x"],
        "B_w1": _B_in["w1"],
        "B_b1": _B_in["b1"],
        "B_w2": _B_in["w2"],
        "B_b2": _B_in["b2"],
    }

def reference(A_x, A_wqkv, A_wo, B_x, B_w1, B_b1, B_w2, B_b2):
    def _A_ref(x, wqkv, wo):
        B, S, D = x.shape
        H = 32; Dh = D // H
        qkv = (lambda x, *d: x.transpose(*d))((x @ wqkv).reshape(B, S, 3, H, Dh), 2, 0, 3, 1, 4)
        q, k, v = qkv[0], qkv[1], qkv[2]
        phi = lambda t: jnp.where(t > 0, t + 1, jnp.exp(t)) + 1e-6
        pq, pk = phi(q), phi(k)
        kv = jnp.einsum("bhsd,bhse->bhde", pk, v)
        z = jnp.einsum("bhsd->bhd", pk)
        num = jnp.einsum("bhqd,bhde->bhqe", pq, kv)
        den = jnp.einsum("bhqd,bhd->bhq", pq, z)[..., None] + 1e-6
        o = num / den
        return (lambda x, *d: x.transpose(*d))(o, 0, 2, 1, 3).reshape(B, S, D) @ wo

    def _B_ref(x, w1, b1, w2, b2):
        h = jnp.einsum("bsd,df->bsf", x, w1) + b1
        zero = jnp.zeros_like(h)
        r = jnp.where(h > zero, h, zero)
        h = r * r
        out = jnp.einsum("bsf,fd->bsd", h, w2) + b2
        return out

    x = A_x
    h = x + _A_ref(_layernorm(x, axis=-1), A_wqkv, A_wo)
    h2 = h + _B_ref(_layernorm(h, axis=-1), B_w1, B_b1, B_w2, B_b2)
    return h2
```

```python
import functools
import numpy as np
import jax
import jax.numpy as jnp
from jax import lax
from jax.experimental import pallas as pl
from jax.experimental.pallas import tpu as pltpu

S, D, H, F = 2048, 576, 32, 4608
DH = D // H
NN = (((1,), (0,)), ((), ()))
NT = (((1,), (1,)), ((), ()))
BF, F32 = jnp.bfloat16, jnp.float32


def _dot(a, b, dims=NN):
    return lax.dot_general(a, b, dims, preferred_element_type=F32)


def _phi(t):
    return jnp.where(t > 0, t + 1.0, jnp.exp(t)) + 1e-6


def _ln_t(x):
    m = jnp.sum(x, axis=0, keepdims=True) * (1.0 / D)
    xc = x - m
    v = jnp.sum(xc * xc, axis=0, keepdims=True) * (1.0 / D)
    return xc * lax.rsqrt(v + 1e-5)


def _expand_heads(r, T):
    sub = lax.broadcasted_iota(jnp.int32, (8, T), 0)
    bc = [jnp.broadcast_to(r[h:h + 1, :], (8, T)) for h in range(H)]
    pieces = []
    for i in range(D // 8):
        h0, h1 = (8 * i) // DH, (8 * i + 7) // DH
        if h0 == h1:
            pieces.append(bc[h0])
        else:
            pieces.append(jnp.where(sub < (h1 * DH - 8 * i), bc[h0], bc[h1]))
    return jnp.concatenate(pieces, axis=0)


def make(T1=512, T2=512, TF=512, dbg=None):
    n1, n2, nf = S // T1, S // T2, S // TF

    def kern(xT_h, wqkv_h, wo_h, w1_h, b1_h, w2T_h, b2_h, out_h,
             xT, wqkv, wo, w1, b1, w2T, b2,
             wT, woT, xnT, GT, MT, ZT, lnS, hT, b2c, outv, sem, osem):
        cp_x = [pltpu.make_async_copy(xT_h.at[:, pl.ds(i * T1, T1)], xT.at[:, pl.ds(i * T1, T1)], sem.at[i])
                for i in range(n1)]
        cp_wqkv = pltpu.make_async_copy(wqkv_h, wqkv, sem.at[n1])
        cp_wo = pltpu.make_async_copy(wo_h, wo, sem.at[n1 + 1])
        cp_w1 = pltpu.make_async_copy(w1_h, w1, sem.at[n1 + 2])
        cp_w2 = pltpu.make_async_copy(w2T_h, w2T, sem.at[n1 + 3])
        cp_b1 = pltpu.make_async_copy(b1_h, b1, sem.at[n1 + 4])
        cp_b2 = pltpu.make_async_copy(b2_h, b2, sem.at[n1 + 5])
        cp_wqkv.start()
        for c in cp_x:
            c.start()
        cp_wo.start()
        cp_b1.start()
        cp_b2.start()

        rows = lax.broadcasted_iota(jnp.int32, (16, S), 0)
        xnT[pl.ds(D, 16), :] = jnp.where(rows == 0, 1.0, 0.0).astype(BF)

        cp_wqkv.wait()
        wT[...] = wqkv[...].T

        for i in range(n1):
            cs = pl.ds(i * T1, T1)
            cp_x[i].wait()
            if i == min(1, n1 - 1):
                cp_w1.start()
                cp_w2.start()
            xn = _ln_t(xT[:, cs].astype(F32)).astype(BF)
            xnT[pl.ds(0, D), cs] = xn
            pk = _phi(_dot(wT[pl.ds(D, D), :], xn)).astype(BF)
            g = _dot(xnT[:, cs], pk, NT)
            if i == 0:
                GT[...] = g
            else:
                GT[...] += g

        cp_wo.wait()
        woT[...] = wo[...].T
        cp_b2.wait()
        b2c[...] = jnp.broadcast_to(b2[...].reshape(1, D).astype(F32), (128, D)).T
        g = GT[...]
        z = g[D:D + 1, :]
        kvT = _dot(wT[pl.ds(2 * D, D), :], g[:D, :].astype(BF))
        e_id = lax.broadcasted_iota(jnp.int32, (D, D), 0)
        d_id = lax.broadcasted_iota(jnp.int32, (D, D), 1)
        same = ((e_id * 3641) >> 16) == ((d_id * 3641) >> 16)
        kvT = jnp.where(same, kvT, 0.0).astype(BF)
        MT[...] = _dot(woT[...], kvT).astype(BF)
        h_id = lax.broadcasted_iota(jnp.int32, (H, D), 0)
        d_id2 = lax.broadcasted_iota(jnp.int32, (H, D), 1)
        ZT[...] = jnp.where(((d_id2 * 3641) >> 16) == h_id, z, 0.0).astype(BF)

        for i in range(n2):
            cs = pl.ds(i * T2, T2)
            pq = _phi(_dot(wT[pl.ds(0, D), :], xnT[pl.ds(0, D), cs]))
            den = _dot(ZT[...], pq.astype(BF)) + 1e-6
            r = 1.0 / den
            pqs = (pq * _expand_heads(r, T2)).astype(BF)
            h = xT[:, cs].astype(F32) + _dot(MT[...], pqs)
            ln = _ln_t(h).astype(BF)
            lnS[pl.ds(i * T2, T2), :] = ln.T
            hT[:, cs] = h + jnp.tile(b2c[...], (1, T2 // 128))

        cp_w1.wait()
        cp_w2.wait()
        cp_b1.wait()

        def ffn(i, _):
            c0 = pl.multiple_of(i * TF, TF)
            cs = pl.ds(c0, TF)
            a = _dot(lnS[cs, :], w1[...]) + b1[...].reshape(1, F).astype(F32)
            a = jnp.maximum(a, 0.0)
            a = (a * a).astype(BF)
            o = _dot(w2T[...], a, NT) + hT[:, cs]
            outv[:, cs] = o.astype(BF)
            pltpu.make_async_copy(outv.at[:, cs], out_h.at[:, cs], osem.at[i]).start()
            return 0

        lax.fori_loop(0, nf, ffn, 0)
        for i in range(nf):
            cs = pl.ds(i * TF, TF)
            pltpu.make_async_copy(outv.at[:, cs], out_h.at[:, cs], osem.at[i]).wait()

    def fn(A_x, A_wqkv, A_wo, B_x, B_w1, B_b1, B_w2, B_b2):
        any_spec = pl.BlockSpec(memory_space=pl.ANY)
        outT = pl.pallas_call(
            kern,
            out_shape=jax.ShapeDtypeStruct((D, S), BF),
            in_specs=[any_spec] * 7,
            out_specs=any_spec,
            scratch_shapes=[
                pltpu.VMEM((D, S), BF),
                pltpu.VMEM((D, 3 * D), BF),
                pltpu.VMEM((D, D), BF),
                pltpu.VMEM((D, F), BF),
                pltpu.VMEM((F,), BF),
                pltpu.VMEM((D, F), BF),
                pltpu.VMEM((D,), BF),
                pltpu.VMEM((3 * D, D), BF),
                pltpu.VMEM((D, D), BF),
                pltpu.VMEM((D + 16, S), BF),
                pltpu.VMEM((D + 16, D), F32),
                pltpu.VMEM((D, D), BF),
                pltpu.VMEM((H, D), BF),
                pltpu.VMEM((S, D), BF),
                pltpu.VMEM((D, S), F32),
                pltpu.VMEM((D, 128), F32),
                pltpu.VMEM((D, S), BF),
                pltpu.SemaphoreType.DMA((n1 + 6,)),
                pltpu.SemaphoreType.DMA((nf,)),
            ],
            compiler_params=pltpu.CompilerParams(vmem_limit_bytes=100 * 1024 * 1024),
            name=f"fused_{T1}_{T2}_{TF}",
        )(A_x[0].T, A_wqkv, A_wo, B_w1, B_b1, B_w2.T, B_b2)
        return outT.T[None]

    return fn


SPECS = [jax.ShapeDtypeStruct(s, BF) for s in
         [(1, S, D), (D, 3 * D), (D, D), (1, S, D), (D, F), (F,), (F, D), (D,)]]


@jax.jit
def pallas_sequential_preLN__linear_attn_block__dense_activation_squared_relu__prompt_kernel(
    A_x, A_wqkv, A_wo, B_x, B_w1, B_b1, B_w2, B_b2):
    return make()(A_x, A_wqkv, A_wo, B_x, B_w1, B_b1, B_w2, B_b2)
```

```python
import contextlib
import numpy as np
import jax
import jax.numpy as jnp
from jax import lax
from jax.experimental import pallas as pl
from jax.experimental.pallas import tpu as pltpu

S, D, H, F = 2048, 576, 32, 4608
DH = D // H
DP = 640
NN = (((1,), (0,)), ((), ()))
NT = (((1,), (1,)), ((), ()))
BF, F32 = jnp.bfloat16, jnp.float32


def _dot(a, b, dims=NN):
    return lax.dot_general(a, b, dims, preferred_element_type=F32)


def _phi(t):
    return jnp.where(t > 0, t + 1.0, jnp.exp(t)) + 1e-6


def _ln_t(x):
    m = jnp.sum(x, axis=0, keepdims=True) * (1.0 / D)
    xc = x - m
    v = jnp.sum(xc * xc, axis=0, keepdims=True) * (1.0 / D)
    return xc * lax.rsqrt(v + 1e-5)


def _expand_heads(r):
    T = r.shape[1]
    sub = lax.broadcasted_iota(jnp.int32, (8, T), 0)
    bc = [jnp.broadcast_to(r[h:h + 1, :], (8, T)) for h in range(H)]
    pieces = []
    for i in range(D // 8):
        h0, h1 = (8 * i) // DH, (8 * i + 7) // DH
        if h0 == h1:
            pieces.append(bc[h0])
        else:
            pieces.append(jnp.where(sub < (h1 * DH - 8 * i), bc[h0], bc[h1]))
    return jnp.concatenate(pieces, axis=0)


def _head(idx):
    return (idx * 3641) >> 16


RJ = [(0, 144), (112, 272), (240, 400), (368, 528), (496, 576)]


def make(T1S=(512, 512, 1024), T2=2048, TF=256, scopes=False, lnblk=128, ln2blk=None, wrap=1,
         barrier_at=(0, 1), wq_at=0, FC=F, RC=1, nobc=False, nosc=False, gtail=False):
    n1 = len(T1S)
    o1 = [sum(T1S[:i]) for i in range(n1)]
    assert sum(T1S) == S
    n2, nf = S // T2, S // TF

    def scope(name):
        return jax.named_scope(name) if scopes else contextlib.nullcontext()

    def kern(*refs):
        if wrap == 0:
            kern_body(*refs)
        else:
            pl.when(pl.program_id(0) == 0)(lambda: kern_body(*refs))

    def kern_body(xT_h, wqkv_h, wo_h, w1_h, b1_h, w2T_h, b2_h, out_h,
                  xT, wqkv, wo, w1, b1, w2T, b2,
                  wT, xnT, G, GT2, Gb, MT, ZT, lnS, hT, b2c, outv, sem):
        def xcp(i):
            cs = pl.ds(o1[i], T1S[i])
            return pltpu.make_async_copy(xT_h.at[:, cs], xT.at[:, cs], sem.at[i + 1 if i else 0])
        def wcp(c0, n, s):
            cs = pl.ds(c0, n)
            return pltpu.make_async_copy(wqkv_h.at[:, cs], wqkv.at[:, cs], sem.at[s])
        cp_x = [xcp(i) for i in range(n1)]
        cp_wk = wcp(512, 640, 1)
        cp_wq = wcp(0, 512, wq_at + 2)
        cp_b2 = pltpu.make_async_copy(b2_h, b2, sem.at[wq_at + 2])
        cp_wv = wcp(1152, 576, n1)
        cp_wo = pltpu.make_async_copy(wo_h, wo, sem.at[n1])
        cp_w1 = pltpu.make_async_copy(w1_h, w1, sem.at[n1 + 1])
        cp_w2 = pltpu.make_async_copy(w2T_h, w2T, sem.at[n1 + 1])
        cp_b1 = pltpu.make_async_copy(b1_h, b1, sem.at[n1 + 1])
        cp_x[0].start()
        cp_wk.start()
        cp_x[1].start()
        cp_wq.start()
        cp_b2.start()
        for c in cp_x[2:]:
            c.start()
        cp_wv.start()
        cp_wo.start()
        cp_b1.start()
        cp_w1.start()
        cp_w2.start()

        rows = lax.broadcasted_iota(jnp.int32, (DP - D, S), 0)
        xnT[pl.ds(D, DP - D), :] = jnp.where(rows == 0, 1.0, 0.0).astype(BF)

        def ln1(i):
            for b in range(T1S[i] // lnblk):
                cs = pl.ds(o1[i] + b * lnblk, lnblk)
                xnT[pl.ds(0, D), cs] = _ln_t(xT[:, cs].astype(F32)).astype(BF)

        pks = {}
        def kproj(i):
            cs = pl.ds(o1[i], T1S[i])
            pks[i] = _phi(_dot(wT[pl.ds(D, D), :], xnT[pl.ds(0, D), cs])).astype(BF)
        def gacc(i):
            cs = pl.ds(o1[i], T1S[i])
            pk = pks.pop(i)
            if gtail:
                g = _dot(pk, xnT[pl.ds(0, 512), cs], NT)
                gt = _dot(xnT[pl.ds(512, 80), cs], pk, NT)
                if i == 0:
                    G[:, pl.ds(0, 512)] = g
                    GT2[...] = gt
                else:
                    G[:, pl.ds(0, 512)] += g
                    GT2[...] += gt
            else:
                g = _dot(pk, xnT[:, cs], NT)
                if i == 0:
                    G[...] = g
                else:
                    G[...] += g

        with scope("w_x0"):
            cp_x[0].wait()
        ln1(0)
        with scope("w_wk"):
            cp_wk.wait()
        wT[pl.ds(512, 640), :] = wqkv[:, pl.ds(512, 640)].T
        for i in range(n1):
            kproj(i)
            if i + 1 < n1:
                with scope(f"w_x{i+1}"):
                    cp_x[i + 1].wait()
                    if i == wq_at:
                        cp_wq.wait(); cp_b2.wait()
                    if i + 1 == n1 - 1:
                        cp_wv.wait(); cp_wo.wait()
                ln1(i + 1)
                if i == wq_at:
                    wT[pl.ds(0, 512), :] = wqkv[:, pl.ds(0, 512)].T
                    b2c[...] = jnp.broadcast_to(b2[...].reshape(1, D).astype(F32), (128, D)).T
            gacc(i)

        if gtail:
            gt2 = GT2[...]
            Gb[:, pl.ds(0, 512)] = G[:, pl.ds(0, 512)].astype(BF)
            Gb[:, pl.ds(512, 64)] = gt2[0:64, :].T.astype(BF)
        else:
            Gb[...] = G[:, pl.ds(0, D)].astype(BF)
        Mp = []
        for j, (r0, r1) in enumerate(RJ):
            w = min(128, D - 128 * j)
            kv = _dot(Gb[pl.ds(r0, r1 - r0), :], wqkv[:, pl.ds(2 * D + 128 * j, w)])
            d_id = lax.broadcasted_iota(jnp.int32, (r1 - r0, w), 0) + r0
            e_id = lax.broadcasted_iota(jnp.int32, (r1 - r0, w), 1) + 128 * j
            kv = jnp.where(_head(d_id) == _head(e_id), kv, 0.0).astype(BF)
            Mp.append(_dot(kv, wo[pl.ds(128 * j, w), :]))
        pieces = []
        bounds = sorted(set([r for rr in RJ for r in rr]))
        for a, b in zip(bounds[:-1], bounds[1:]):
            acc = None
            for j, (r0, r1) in enumerate(RJ):
                if r0 <= a and b <= r1:
                    p = Mp[j][a - r0:b - r0, :]
                    acc = p if acc is None else acc + p
            pieces.append(acc)
        M = jnp.concatenate(pieces, axis=0)
        MT[...] = M.astype(BF).T
        if gtail:
            z = gt2[64:65, :]
        else:
            z = G[:, pl.ds(512, 128)].T[64:65, :]
        h_id = lax.broadcasted_iota(jnp.int32, (H, D), 0)
        d_id2 = lax.broadcasted_iota(jnp.int32, (H, D), 1)
        ZT[...] = jnp.where(_head(d_id2) == h_id, z, 0.0).astype(BF)

        def ln2(c0, slot):
            blk = ln2blk or TF
            for b in range(TF // blk):
                cs = pl.ds(c0 + b * blk, blk)
                lnS[slot, pl.ds(b * blk, blk), :] = _ln_t(hT[:, cs]).astype(BF).T

        for i in range(n2):
            cs = pl.ds(i * T2, T2)
            pq = _phi(_dot(wT[pl.ds(0, D), :], xnT[pl.ds(0, D), cs]))
            den = _dot(ZT[...], pq.astype(BF)) + 1e-6
            r = 1.0 / den
            pqs = (pq * _expand_heads(r)).astype(BF)
            hT[:, cs] = xT[:, cs].astype(F32) + _dot(MT[...], pqs)
        ln2(0, 0)

        with scope("w_w1w2"):
            cp_w1.wait()
            cp_w2.wait()
            cp_b1.wait()

        def out_cp(i, r):
            rs = pl.ds(r * (D // RC), D // RC)
            cs = pl.ds(pl.multiple_of(i * TF, TF), TF) if not isinstance(i, int) else pl.ds(i * TF, TF)
            return pltpu.make_async_copy(outv.at[rs, cs], out_h.at[rs, cs], sem.at[n1 + 2])

        def ffn(i, _):
            cs = pl.ds(pl.multiple_of(i * TF, TF), TF)
            nxt = lax.rem(i + 1, nf)
            ln = lnS[lax.rem(i, 2)]
            b1r = b1[...].reshape(1, F).astype(F32)
            a = _dot(ln, w1[...]) + b1r
            a = jnp.maximum(a, 0.0)
            a = (a * a).astype(BF)
            ln2(pl.multiple_of(nxt * TF, TF), lax.rem(i + 1, 2))
            for r in range(RC):
                rs = pl.ds(r * (D // RC), D // RC)
                o = _dot(w2T[rs, :], a, NT) + hT[rs, cs] + jnp.tile(b2c[rs, :], (1, TF // 128))
                outv[rs, cs] = o.astype(BF)
                out_cp(i, r).start()
            return 0

        with scope("ffn"):
            lax.fori_loop(0, nf, ffn, 0)
        with scope("w_out"):
            pltpu.make_async_copy(outv, out_h, sem.at[n1 + 2]).wait()

    def fn(A_x, A_wqkv, A_wo, B_x, B_w1, B_b1, B_w2, B_b2):
        any_spec = pl.BlockSpec(memory_space=pl.ANY)
        outT = pl.pallas_call(
            kern,
            grid=(2,) if wrap else (),
            out_shape=jax.ShapeDtypeStruct((D, S), BF),
            in_specs=[any_spec] * 7,
            out_specs=any_spec,
            scratch_shapes=[
                pltpu.VMEM((D, S), BF),
                pltpu.VMEM((D, 3 * D), BF),
                pltpu.VMEM((D, D), BF),
                pltpu.VMEM((D, F), BF),
                pltpu.VMEM((F,), BF),
                pltpu.VMEM((D, F), BF),
                pltpu.VMEM((D,), BF),
                pltpu.VMEM((2 * D, D), BF),
                pltpu.VMEM((DP, S), BF),
                pltpu.VMEM((D, DP), F32),
                pltpu.VMEM((80, D), F32),
                pltpu.VMEM((D, D), BF),
                pltpu.VMEM((D, D), BF),
                pltpu.VMEM((H, D), BF),
                pltpu.VMEM((2, TF, D), BF),
                pltpu.VMEM((D, S), F32),
                pltpu.VMEM((D, 128), F32),
                pltpu.VMEM((D, S), BF),
                pltpu.SemaphoreType.DMA((n1 + 3,)),
            ],
            compiler_params=pltpu.CompilerParams(vmem_limit_bytes=100 * 1024 * 1024, disable_bounds_checks=nobc, disable_semaphore_checks=nosc),
            name="fused",
        )(A_x[0].T, A_wqkv, A_wo, B_w1, B_b1, B_w2.T, B_b2)
        return outT.T[None]

    return fn


SPECS = [jax.ShapeDtypeStruct(s, BF) for s in
         [(1, S, D), (D, 3 * D), (D, D), (1, S, D), (D, F), (F,), (F, D), (D,)]]


@jax.jit
def pallas_sequential_preLN__linear_attn_block__dense_activation_squared_relu__prompt_kernel(
    A_x, A_wqkv, A_wo, B_x, B_w1, B_b1, B_w2, B_b2):
    return make(RC=2, wq_at=1, gtail=True)(A_x, A_wqkv, A_wo, B_x, B_w1, B_b1, B_w2, B_b2)
```

```python
import jax
import jax.numpy as jnp
from jax import lax
from jax.experimental import pallas as pl
from jax.experimental.pallas import tpu as pltpu

S, D, H, F = 2048, 576, 32, 4608
DH = D // H
DP = 640
T1S = (512, 512, 1024)
KSPLIT = 384
TF = 256
RC = 2
PAD = 128

NN = (((1,), (0,)), ((), ()))
NT = (((1,), (1,)), ((), ()))
BF, F32 = jnp.bfloat16, jnp.float32

RJ = ((0, 144), (112, 272), (240, 400), (368, 528), (496, 576))


def _dot(a, b, dims=NN):
    return lax.dot_general(a, b, dims, preferred_element_type=F32)


def _phi(t):
    return jnp.where(t > 0, t + 1.0, jnp.exp(t)) + 1e-6


def _ln_t(x):
    m = jnp.sum(x, axis=0, keepdims=True) * (1.0 / D)
    xc = x - m
    v = jnp.sum(xc * xc, axis=0, keepdims=True) * (1.0 / D)
    return xc * lax.rsqrt(v + 1e-5)


def _expand_heads(r):
    t = r.shape[1]
    sub = lax.broadcasted_iota(jnp.int32, (8, t), 0)
    bc = [jnp.broadcast_to(r[h:h + 1, :], (8, t)) for h in range(H)]
    pieces = []
    for i in range(D // 8):
        h0, h1 = (8 * i) // DH, (8 * i + 7) // DH
        if h0 == h1:
            pieces.append(bc[h0])
        else:
            pieces.append(jnp.where(sub < (h1 * DH - 8 * i), bc[h0], bc[h1]))
    return jnp.concatenate(pieces, axis=0)


def _head(idx):
    return (idx * 3641) >> 16


class _Tiled:
    def __init__(self, ref, lead=()):
        self.ref, self.lead = ref, tuple(lead)

    @staticmethod
    def _tiles(cs):
        c0, c1 = cs.start, cs.start + cs.size
        return [(c, max(c0, 128 * c) - 128 * c, min(c1, 128 * c + 128) - 128 * c)
                for c in range(c0 // 128, (c1 + 127) // 128)]

    def __getitem__(self, idx):
        rs, cs = idx
        ps = [self.ref[(*self.lead, c, rs, pl.ds(a, b - a))] for c, a, b in self._tiles(cs)]
        return ps[0] if len(ps) == 1 else jnp.concatenate(ps, axis=1)

    def __setitem__(self, idx, v):
        rs, cs = idx
        off = 0
        for c, a, b in self._tiles(cs):
            self.ref[(*self.lead, c, rs, pl.ds(a, b - a))] = v[:, off:off + b - a]
            off += b - a


def _block(xT_h, wqkv_h, wo_h, w1_h, b1_h, w2T_h, b2_h, out_h,
           xT, wqkv, wo, w1, b1, w2T, b2,
           wT_r, xn_r, G, GT2, Gb_r, MT_r, ZT, ln_r, hT, b2c, outv, sem):
    wT, xnT, Gb, MT = _Tiled(wT_r), _Tiled(xn_r), _Tiled(Gb_r), _Tiled(MT_r)
    ALL = pl.ds(0, D)
    n1 = len(T1S)
    o1 = [sum(T1S[:i]) for i in range(n1)]
    nf = S // TF

    def x_cp(i, s):
        cs = pl.ds(o1[i], T1S[i])
        return pltpu.make_async_copy(xT_h.at[:, cs], xT.at[:, cs], sem.at[s])

    def w_cp(r0, nr, c0, nc, s):
        rs, cs = pl.ds(r0, nr), pl.ds(c0, nc)
        return pltpu.make_async_copy(wqkv_h.at[rs, cs], wqkv.at[rs, cs], sem.at[s])

    cp_x = [x_cp(0, 0), x_cp(1, 3), x_cp(2, 4)]
    cp_wka = w_cp(0, KSPLIT, 512, 640, 1)
    cp_wkb = w_cp(KSPLIT, D - KSPLIT, 512, 640, 2)
    cp_wq = w_cp(0, D, 0, 512, 4)
    cp_wv = w_cp(0, D, 1152, 576, 4)
    cp_wo = pltpu.make_async_copy(wo_h, wo, sem.at[4])
    cp_b2 = pltpu.make_async_copy(b2_h, b2, sem.at[4])
    cp_w1 = pltpu.make_async_copy(w1_h, w1, sem.at[5])
    cp_w2 = pltpu.make_async_copy(w2T_h, w2T, sem.at[5])
    cp_b1 = pltpu.make_async_copy(b1_h, b1, sem.at[5])
    for c in (cp_x[0], cp_wka, cp_wkb, cp_x[1], cp_wq, cp_b2, cp_x[2], cp_wv, cp_wo,
              cp_b1, cp_w1, cp_w2):
        c.start()

    rows = lax.broadcasted_iota(jnp.int32, (DP - D, S), 0)
    xnT[pl.ds(D, DP - D), pl.ds(0, S)] = jnp.where(rows == 0, 1.0, 0.0).astype(BF)

    def ln1(i):
        for b in range(T1S[i] // 128):
            cs = pl.ds(o1[i] + b * 128, 128)
            xnT[ALL, cs] = _ln_t(xT[:, cs].astype(F32)).astype(BF)

    def wk_t(r0, nr):
        wT[pl.ds(512, 640), pl.ds(r0, nr)] = (
            wqkv[pl.ds(r0, nr), pl.ds(512, 640)].astype(F32).T.astype(BF))

    cp_x[0].wait()
    ln1(0)
    cp_wka.wait()
    wk_t(0, KSPLIT)
    c0 = pl.ds(0, T1S[0])
    ka, kb = pl.ds(0, KSPLIT), pl.ds(KSPLIT, D - KSPLIT)
    hT[:, c0] = _dot(wT[pl.ds(D, D), ka], xnT[ka, c0])
    cp_wkb.wait()
    cp_x[1].wait()
    wk_t(KSPLIT, D - KSPLIT)
    for i in range(n1):
        cs = pl.ds(o1[i], T1S[i])
        if i == 0:
            k = hT[:, cs] + _dot(wT[pl.ds(D, D), kb], xnT[kb, cs])
        else:
            k = _dot(wT[pl.ds(D, D), ALL], xnT[ALL, cs])
        pk = _phi(k).astype(BF)
        if i + 1 < n1:
            if i + 1 == n1 - 1:
                for c in (cp_x[2], cp_wq, cp_b2, cp_wv, cp_wo):
                    c.wait()
            ln1(i + 1)
            if i + 1 == n1 - 1:
                wT[pl.ds(0, 512), ALL] = wqkv[:, pl.ds(0, 512)].T
                b2c[...] = jnp.broadcast_to(b2[...].reshape(1, D).astype(F32), (128, D)).T
        g = _dot(pk, xnT[pl.ds(0, 512), cs], NT)
        gt = _dot(xnT[pl.ds(512, 80), cs], pk, NT)
        if i == 0:
            G[...] = g
            GT2[...] = gt
        else:
            G[...] += g
            GT2[...] += gt

    gt2 = GT2[...]
    Gb[ALL, pl.ds(0, 512)] = G[...].astype(BF)
    Gb[ALL, pl.ds(512, 64)] = gt2[0:64, :].T.astype(BF)
    mp = []
    for j, (r0, r1) in enumerate(RJ):
        w = min(128, D - 128 * j)
        kv = _dot(Gb[pl.ds(r0, r1 - r0), ALL], wqkv[:, pl.ds(2 * D + 128 * j, w)])
        d_id = lax.broadcasted_iota(jnp.int32, (r1 - r0, w), 0) + r0
        e_id = lax.broadcasted_iota(jnp.int32, (r1 - r0, w), 1) + 128 * j
        kv = jnp.where(_head(d_id) == _head(e_id), kv, 0.0).astype(BF)
        mp.append(_dot(kv, wo[pl.ds(128 * j, w), :]))
    pieces = []
    bounds = sorted({r for rr in RJ for r in rr})
    for a, b in zip(bounds[:-1], bounds[1:]):
        acc = None
        for j, (r0, r1) in enumerate(RJ):
            if r0 <= a and b <= r1:
                p = mp[j][a - r0:b - r0, :]
                acc = p if acc is None else acc + p
        pieces.append(acc)
    MT[ALL, ALL] = jnp.concatenate(pieces, axis=0).astype(BF).T
    h_id = lax.broadcasted_iota(jnp.int32, (H, D), 0)
    d_id = lax.broadcasted_iota(jnp.int32, (H, D), 1)
    ZT[...] = jnp.where(_head(d_id) == h_id, gt2[64:65, :], 0.0).astype(BF)

    cs = pl.ds(0, S)
    pq = _phi(_dot(wT[ALL, ALL], xnT[ALL, cs]))
    den = _dot(ZT[...], pq.astype(BF)) + 1e-6
    pqs = (pq * _expand_heads(1.0 / den)).astype(BF)
    hT[:, cs] = xT[:, cs].astype(F32) + _dot(MT[ALL, ALL], pqs)

    def ln2(t0, slot):
        _Tiled(ln_r, (slot,))[pl.ds(0, TF), ALL] = _ln_t(hT[:, pl.ds(t0, TF)]).astype(BF).T

    ln2(0, 0)

    cp_w1.wait()
    cp_w2.wait()
    cp_b1.wait()

    def ffn(i, carry):
        cs = pl.ds(pl.multiple_of(i * TF, TF), TF)
        ln = _Tiled(ln_r, (lax.rem(i, 2),))[pl.ds(0, TF), ALL]
        a = _dot(ln, w1[...]) + b1[...].reshape(1, F).astype(F32)
        a = jnp.maximum(a, 0.0)
        a = (a * a).astype(BF)
        ln2(pl.multiple_of(lax.rem(i + 1, nf) * TF, TF), lax.rem(i + 1, 2))
        for r in range(RC):
            rs = pl.ds(r * (D // RC), D // RC)
            o = _dot(w2T[rs, :], a, NT) + hT[rs, cs] + jnp.tile(b2c[rs, :], (1, TF // 128))
            outv[rs, cs] = o.astype(BF)
            pltpu.make_async_copy(outv.at[rs, cs], out_h.at[rs, cs], sem.at[6]).start()
        return carry

    lax.fori_loop(0, nf, ffn, 0)
    pltpu.make_async_copy(outv, outv, sem.at[6]).wait()


def _kernel(*refs):
    pl.when(pl.program_id(0) == 0)(lambda: _block(*refs))


@jax.jit
def pallas_sequential_preLN__linear_attn_block__dense_activation_squared_relu__prompt_kernel(
    A_x: jax.Array,
    A_wqkv: jax.Array,
    A_wo: jax.Array,
    B_x: jax.Array,
    B_w1: jax.Array,
    B_b1: jax.Array,
    B_w2: jax.Array,
    B_b2: jax.Array,
):
    del B_x
    any_spec = pl.BlockSpec(memory_space=pl.ANY)
    outT = pl.pallas_call(
        _kernel,
        grid=(2,),
        out_shape=jax.ShapeDtypeStruct((D, S), BF),
        in_specs=[any_spec] * 7,
        out_specs=any_spec,
        scratch_shapes=[
            pltpu.VMEM((D, S + PAD), BF),
            pltpu.VMEM((D, 3 * D), BF),
            pltpu.VMEM((D, D), BF),
            pltpu.VMEM((D, F), BF),
            pltpu.VMEM((F,), BF),
            pltpu.VMEM((D, F), BF),
            pltpu.VMEM((D,), BF),
            pltpu.VMEM((5, 2 * D, 128), BF),
            pltpu.VMEM((S // 128, DP, 128), BF),
            pltpu.VMEM((D, 512), F32),
            pltpu.VMEM((80, D), F32),
            pltpu.VMEM((5, D, 128), BF),
            pltpu.VMEM((5, D, 128), BF),
            pltpu.VMEM((H, D), BF),
            pltpu.VMEM((2, 5, TF, 128), BF),
            pltpu.VMEM((D, S + PAD), F32),
            pltpu.VMEM((D, 128), F32),
            pltpu.VMEM((D, S), BF),
            pltpu.SemaphoreType.DMA((7,)),
        ],
        compiler_params=pltpu.CompilerParams(vmem_limit_bytes=100 * 1024 * 1024),
        name="preln_linattn_sqrelu_ffn",
    )(A_x[0].T, A_wqkv, A_wo, B_w1, B_b1, B_w2.T, B_b2)
    return outT.T[None]
```

```python
import jax
import jax.numpy as jnp
from jax import lax
from jax.experimental import pallas as pl
from jax.experimental.pallas import tpu as pltpu

S, D, H, F = 2048, 576, 32, 4608
DH = D // H
DP = 640
T1S = (512, 512, 1024)
KSPLIT = 384
TF = 256
RC = 2
PAD = 128

NN = (((1,), (0,)), ((), ()))
NT = (((1,), (1,)), ((), ()))
BF, F32 = jnp.bfloat16, jnp.float32

RJ = ((0, 144), (112, 272), (240, 400), (368, 528), (496, 576))


def _dot(a, b, dims=NN):
    return lax.dot_general(a, b, dims, preferred_element_type=F32)


def _phi(t):
    return jnp.where(t > 0, t + 1.0, jnp.exp(t)) + 1e-6


def _ln_t(x):
    m = jnp.sum(x, axis=0, keepdims=True) * (1.0 / D)
    xc = x - m
    v = jnp.sum(xc * xc, axis=0, keepdims=True) * (1.0 / D)
    return xc * lax.rsqrt(v + 1e-5)


def _expand_heads(r):
    t = r.shape[1]
    sub = lax.broadcasted_iota(jnp.int32, (8, t), 0)
    bc = [jnp.broadcast_to(r[h:h + 1, :], (8, t)) for h in range(H)]
    pieces = []
    for i in range(D // 8):
        h0, h1 = (8 * i) // DH, (8 * i + 7) // DH
        if h0 == h1:
            pieces.append(bc[h0])
        else:
            pieces.append(jnp.where(sub < (h1 * DH - 8 * i), bc[h0], bc[h1]))
    return jnp.concatenate(pieces, axis=0)


def _head(idx):
    return (idx * 3641) >> 16


class _Tiled:
    def __init__(self, ref, lead=()):
        self.ref, self.lead = ref, tuple(lead)

    @staticmethod
    def _tiles(cs):
        c0, c1 = cs.start, cs.start + cs.size
        return [(c, max(c0, 128 * c) - 128 * c, min(c1, 128 * c + 128) - 128 * c)
                for c in range(c0 // 128, (c1 + 127) // 128)]

    def __getitem__(self, idx):
        rs, cs = idx
        ps = [self.ref[(*self.lead, c, rs, pl.ds(a, b - a))] for c, a, b in self._tiles(cs)]
        return ps[0] if len(ps) == 1 else jnp.concatenate(ps, axis=1)

    def __setitem__(self, idx, v):
        rs, cs = idx
        off = 0
        for c, a, b in self._tiles(cs):
            self.ref[(*self.lead, c, rs, pl.ds(a, b - a))] = v[:, off:off + b - a]
            off += b - a


def _block(xT_h, wqkv_h, wo_h, w1_h, b1_h, w2T_h, b2_h, out_h,
           xT, wqkv, wo, w1, b1, w2T, b2,
           wT_r, xn_r, G, GT2, Gb_r, MT_r, ZT, ln_r, hT, b2c, outv, sem):
    wT, xnT, Gb, MT = _Tiled(wT_r), _Tiled(xn_r), _Tiled(Gb_r), _Tiled(MT_r)
    ALL = pl.ds(0, D)
    n1 = len(T1S)
    o1 = [sum(T1S[:i]) for i in range(n1)]
    nf = S // TF

    def x_cp(i, s):
        cs = pl.ds(o1[i], T1S[i])
        return pltpu.make_async_copy(xT_h.at[:, cs], xT.at[:, cs], sem.at[s])

    def w_cp(r0, nr, c0, nc, s):
        rs, cs = pl.ds(r0, nr), pl.ds(c0, nc)
        return pltpu.make_async_copy(wqkv_h.at[rs, cs], wqkv.at[rs, cs], sem.at[s])

    cp_x = [x_cp(0, 0), x_cp(1, 3), x_cp(2, 4)]
    cp_wka = w_cp(0, KSPLIT, 512, 640, 1)
    cp_wkb = w_cp(KSPLIT, D - KSPLIT, 512, 640, 2)
    cp_wq = w_cp(0, D, 0, 512, 4)
    cp_wv = w_cp(0, D, 1152, 576, 4)
    cp_wo = pltpu.make_async_copy(wo_h, wo, sem.at[4])
    cp_b2 = pltpu.make_async_copy(b2_h, b2, sem.at[4])
    cp_w1 = pltpu.make_async_copy(w1_h, w1, sem.at[5])
    cp_w2 = pltpu.make_async_copy(w2T_h, w2T, sem.at[5])
    cp_b1 = pltpu.make_async_copy(b1_h, b1, sem.at[5])
    for c in (cp_x[0], cp_wka, cp_wkb, cp_x[1], cp_wq, cp_b2, cp_x[2], cp_wv, cp_wo,
              cp_b1, cp_w1, cp_w2):
        c.start()

    rows = lax.broadcasted_iota(jnp.int32, (DP - D, S), 0)
    xnT[pl.ds(D, DP - D), pl.ds(0, S)] = jnp.where(rows == 0, 1.0, 0.0).astype(BF)

    def ln1(i):
        for b in range(T1S[i] // 128):
            cs = pl.ds(o1[i] + b * 128, 128)
            xnT[ALL, cs] = _ln_t(xT[:, cs].astype(F32)).astype(BF)

    def wk_t(r0, nr):
        wT[pl.ds(512, 640), pl.ds(r0, nr)] = (
            wqkv[pl.ds(r0, nr), pl.ds(512, 640)].astype(F32).T.astype(BF))

    cp_x[0].wait()
    ln1(0)
    cp_wka.wait()
    wk_t(0, KSPLIT)
    c0 = pl.ds(0, T1S[0])
    ka, kb = pl.ds(0, KSPLIT), pl.ds(KSPLIT, D - KSPLIT)
    hT[:, c0] = _dot(wT[pl.ds(D, D), ka], xnT[ka, c0])
    cp_wkb.wait()
    cp_x[1].wait()
    wk_t(KSPLIT, D - KSPLIT)
    for i in range(n1):
        cs = pl.ds(o1[i], T1S[i])
        if i == 0:
            k = hT[:, cs] + _dot(wT[pl.ds(D, D), kb], xnT[kb, cs])
        else:
            k = _dot(wT[pl.ds(D, D), ALL], xnT[ALL, cs])
        pk = _phi(k).astype(BF)
        if i + 1 < n1:
            if i + 1 == n1 - 1:
                for c in (cp_x[2], cp_wq, cp_b2, cp_wv, cp_wo):
                    c.wait()
            ln1(i + 1)
            if i + 1 == n1 - 1:
                wT[pl.ds(0, 512), ALL] = wqkv[:, pl.ds(0, 512)].T
                b2c[...] = jnp.broadcast_to(b2[...].reshape(1, D).astype(F32), (128, D)).T
        g = _dot(pk, xnT[pl.ds(0, 512), cs], NT)
        gt = _dot(xnT[pl.ds(512, 80), cs], pk, NT)
        if i == 0:
            G[...] = g
            GT2[...] = gt
        else:
            G[...] += g
            GT2[...] += gt

    gt2 = GT2[...]
    Gb[ALL, pl.ds(0, 512)] = G[...].astype(BF)
    Gb[ALL, pl.ds(512, 64)] = gt2[0:64, :].T.astype(BF)
    mp = []
    for j, (r0, r1) in enumerate(RJ):
        w = min(128, D - 128 * j)
        kv = _dot(Gb[pl.ds(r0, r1 - r0), ALL], wqkv[:, pl.ds(2 * D + 128 * j, w)])
        d_id = lax.broadcasted_iota(jnp.int32, (r1 - r0, w), 0) + r0
        e_id = lax.broadcasted_iota(jnp.int32, (r1 - r0, w), 1) + 128 * j
        kv = jnp.where(_head(d_id) == _head(e_id), kv, 0.0).astype(BF)
        mp.append(_dot(kv, wo[pl.ds(128 * j, w), :]))
    pieces = []
    bounds = sorted({r for rr in RJ for r in rr})
    for a, b in zip(bounds[:-1], bounds[1:]):
        acc = None
        for j, (r0, r1) in enumerate(RJ):
            if r0 <= a and b <= r1:
                p = mp[j][a - r0:b - r0, :]
                acc = p if acc is None else acc + p
        pieces.append(acc)
    MT[ALL, ALL] = jnp.concatenate(pieces, axis=0).astype(BF).T
    h_id = lax.broadcasted_iota(jnp.int32, (H, D), 0)
    d_id = lax.broadcasted_iota(jnp.int32, (H, D), 1)
    ZT[...] = jnp.where(_head(d_id) == h_id, gt2[64:65, :], 0.0).astype(BF)

    cs = pl.ds(0, S)
    pq = _phi(_dot(wT[ALL, ALL], xnT[ALL, cs]))
    den = _dot(ZT[...], pq.astype(BF)) + 1e-6
    pqs = (pq * _expand_heads(1.0 / den)).astype(BF)
    hT[:, cs] = xT[:, cs].astype(F32) + _dot(MT[ALL, ALL], pqs)

    def ln2(t0, slot):
        _Tiled(ln_r, (slot,))[pl.ds(0, TF), ALL] = _ln_t(hT[:, pl.ds(t0, TF)]).astype(BF).T

    ln2(0, 0)

    cp_w1.wait()
    cp_w2.wait()
    cp_b1.wait()

    def ffn(i, carry):
        cs = pl.ds(pl.multiple_of(i * TF, TF), TF)
        ln = _Tiled(ln_r, (lax.rem(i, 2),))[pl.ds(0, TF), ALL]
        a = _dot(ln, w1[...]) + b1[...].reshape(1, F).astype(F32)
        a = jnp.maximum(a, 0.0)
        a = (a * a).astype(BF)
        ln2(pl.multiple_of(lax.rem(i + 1, nf) * TF, TF), lax.rem(i + 1, 2))
        for r in range(RC):
            rs = pl.ds(r * (D // RC), D // RC)
            o = _dot(w2T[rs, :], a, NT) + hT[rs, cs] + jnp.tile(b2c[rs, :], (1, TF // 128))
            outv[rs, cs] = o.astype(BF)
            pltpu.make_async_copy(outv.at[rs, cs], out_h.at[rs, cs], sem.at[6]).start()
        return carry

    lax.fori_loop(0, nf, ffn, 0)
    pltpu.make_async_copy(outv, outv, sem.at[6]).wait()


def _kernel(*refs):
    pl.when(pl.program_id(0) == 0)(lambda: _block(*refs))


@jax.jit
def pallas_sequential_preLN__linear_attn_block__dense_activation_squared_relu__prompt_kernel(
    A_x: jax.Array,
    A_wqkv: jax.Array,
    A_wo: jax.Array,
    B_x: jax.Array,
    B_w1: jax.Array,
    B_b1: jax.Array,
    B_w2: jax.Array,
    B_b2: jax.Array,
):
    del B_x
    any_spec = pl.BlockSpec(memory_space=pl.ANY)
    outT = pl.pallas_call(
        _kernel,
        grid=(2,),
        out_shape=jax.ShapeDtypeStruct((D, S), BF),
        in_specs=[any_spec] * 7,
        out_specs=any_spec,
        scratch_shapes=[
            pltpu.VMEM((D, S + PAD), BF),
            pltpu.VMEM((D, 3 * D), BF),
            pltpu.VMEM((D, D), BF),
            pltpu.VMEM((D, F), BF),
            pltpu.VMEM((F,), BF),
            pltpu.VMEM((D, F), BF),
            pltpu.VMEM((D,), BF),
            pltpu.VMEM((5, 2 * D, 128), BF),
            pltpu.VMEM((S // 128, DP, 128), BF),
            pltpu.VMEM((D, 512), F32),
            pltpu.VMEM((80, D), F32),
            pltpu.VMEM((5, D, 128), BF),
            pltpu.VMEM((5, D, 128), BF),
            pltpu.VMEM((H, D), BF),
            pltpu.VMEM((2, 5, TF, 128), BF),
            pltpu.VMEM((D, S + PAD), F32),
            pltpu.VMEM((D, 128), F32),
            pltpu.VMEM((D, S), BF),
            pltpu.SemaphoreType.DMA((7,)),
        ],
        compiler_params=pltpu.CompilerParams(
            vmem_limit_bytes=100 * 1024 * 1024,
            disable_bounds_checks=True,
            disable_semaphore_checks=True,
        ),
        name="preln_linattn_sqrelu_ffn",
    )(A_x[0].T, A_wqkv, A_wo, B_w1, B_b1, B_w2.T, B_b2)
    return outT.T[None]
```
